```python
import jax
import jax.numpy as jnp

def _softmax(x, axis=-1):
    return jax.nn.softmax(x, axis=axis)
def _gelu(x):
    return jax.nn.gelu(x, approximate=True)
def _silu(x):
    return jax.nn.silu(x)
def _sigmoid(x):
    return jax.nn.sigmoid(x)
def _layernorm(x, axis=-1, eps=1e-5):
    m = jnp.mean(x, axis=axis, keepdims=True)
    v = jnp.var(x, axis=axis, keepdims=True)
    return (x - m) / jnp.sqrt(v + eps)
def _scatter_add(tgt, idx, src, axis=0):
    return tgt.at[idx].add(src)
def _segment_sum(src, seg, n):
    return jax.ops.segment_sum(src, seg, n)
class _Rng:
    def __init__(self, key):
        self._k = key
    def _next(self):
        self._k, sub = jax.random.split(self._k)
        return sub
    def normal(self, shape):
        return jax.random.normal(self._next(), shape, dtype=jnp.bfloat16)
    def randint(self, lo, hi, shape):
        return jax.random.randint(self._next(), shape, lo, hi, dtype=jnp.int32)
    def uniform(self, shape, lo=0.0, hi=1.0):
        return jax.random.uniform(self._next(), shape, jnp.bfloat16, lo, hi)
    def permutation(self, n):
        return jax.random.permutation(self._next(), n)


kernel_name = 'parallel_sum__gqa_block_cached__moe_arch_mod__decode'

def setup_inputs():
    _rng = _Rng(jax.random.key(int.from_bytes(__import__("os").urandom(4), "little")))
    _w = (lambda a: (lambda t: t.astype(jnp.bfloat16) if jnp.issubdtype(t.dtype, jnp.floating) else t)(jnp.asarray(a)))
    def _A_setup():
        B, Sq, D = 1, 1, 448
        Hq, Hkv, Sk, Dh = 16, 8, 65536, 256
        assert Hq % Hkv == 0, (Hq, Hkv)
        return {
            "x": _w((lambda *s: _rng.normal(s) * 0.05)(B, Sq, D)),
            "k_cache": _w((lambda *s: _rng.normal(s) * 0.05)(B, Hkv, Sk, Dh)),
            "v_cache": _w((lambda *s: _rng.normal(s) * 0.05)(B, Hkv, Sk, Dh)),
            "wq": _w((lambda *s: _rng.normal(s) * 0.05)(D, Hq * Dh) * (D ** -0.5)),
            "wo": _w((lambda *s: _rng.normal(s) * 0.05)(Hq * Dh, D) * ((Hq * Dh) ** -0.5)),
        }
    _A_in = _A_setup()

    def _B_setup():
        B, S, D, F, C = 1, 1, 448, 1792, 1
        return {
            "x": _w((lambda *s: _rng.normal(s) * 0.05)(B, S, D)),
            "w_r": _w((lambda *s: _rng.normal(s) * 0.05)(D)),
            "w_gate": _w((lambda *s: _rng.normal(s) * 0.05)(D, F)),
            "w_up": _w((lambda *s: _rng.normal(s) * 0.05)(D, F)),
            "w_down": _w((lambda *s: _rng.normal(s) * 0.05)(F, D)),
        }
    _B_in = _B_setup()

    return {
        "A_x": _A_in["x"],
        "A_k_cache": _A_in["k_cache"],
        "A_v_cache": _A_in["v_cache"],
        "A_wq": _A_in["wq"],
        "A_wo": _A_in["wo"],
        "B_x": _B_in["x"],
        "B_w_r": _B_in["w_r"],
        "B_w_gate": _B_in["w_gate"],
        "B_w_up": _B_in["w_up"],
        "B_w_down": _B_in["w_down"],
    }

def reference(A_x, A_k_cache, A_v_cache, A_wq, A_wo, B_x, B_w_r, B_w_gate, B_w_up, B_w_down):
    def _A_ref(x, k_cache, v_cache, wq, wo):
        B, Sq, D = x.shape
        Hq, Dh = 16, 256
        Hkv = k_cache.shape[1]
        rep = Hq // Hkv
        q = (lambda x, *d: x.transpose(*d))((x @ wq).reshape(B, Sq, Hq, Dh), 0, 2, 1, 3)
        k = jnp.repeat(k_cache, rep, axis=1)
        v = jnp.repeat(v_cache, rep, axis=1)
        scores = jnp.einsum("bhqd,bhkd->bhqk", q, k) * (Dh ** -0.5)
        p = _softmax(scores, axis=-1)
        o = jnp.einsum("bhqk,bhkd->bhqd", p, v)
        return (lambda x, *d: x.transpose(*d))(o, 0, 2, 1, 3).reshape(B, Sq, Hq * Dh) @ wo

    def _B_ref(x, w_r, w_gate, w_up, w_down):
        B, S, D = x.shape
        C = 1
        r = x @ w_r
        idx = jnp.argsort(-r, axis=-1)[:, :C]
        idx_e = jnp.repeat(idx.reshape(B, C, 1), D, axis=2)
        x_sel = jnp.take_along_axis(x, idx_e, axis=1)
        g = _silu(x_sel @ w_gate)
        u = x_sel @ w_up
        y = (g * u) @ w_down
        r_sel = _sigmoid(jnp.take_along_axis(r, idx, axis=1))
        y = y * r_sel.reshape(B, C, 1)
        b_off = (jnp.arange(B) * S).reshape(B, 1)
        flat_idx = (idx + b_off).reshape(B * C)
        zero = (x * 0.0).reshape(B * S, D)
        upd = _scatter_add(zero, flat_idx, y.reshape(B * C, D), axis=0)
        return x + upd.reshape(B, S, D)

    x = A_x
    xn = _layernorm(x, axis=-1)
    return x + _A_ref(xn, A_k_cache, A_v_cache, A_wq, A_wo) + _B_ref(xn, B_w_r, B_w_gate, B_w_up, B_w_down)
```

```python
import functools

import jax
import jax.numpy as jnp
from jax import lax
import jax.experimental.pallas as pl
import jax.experimental.pallas.tpu as pltpu

D = 448
HQ = 16
HKV = 8
REP = HQ // HKV
SK = 65536
DH = 256
F = 1792
ROWS = 8
EPS = 1e-5

T = 2048
NBUF = 4
NCH = SK // T
TOTAL = HKV * NCH
WD_PIECE = 256
N_WD = F // WD_PIECE

_NT = (((1,), (1,)), ((), ()))


def _kernel(x_hbm, k_hbm, v_hbm, wq_hbm, wot_hbm, wr_hbm, wg_hbm, wu_hbm, wdt_hbm,
            o_ref,
            xbuf, wrbuf, wqbuf, wobuf, wgbuf, wubuf, wdbuf, kbuf, vbuf,
            q_scr, o_scr, m_scr, l_scr, acc_scr,
            kv_sems, w_sems, wd_sems):
    f32 = jnp.float32
    bf16 = jnp.bfloat16

    def kv_copies(i, slot):
        h = i // NCH
        c = i % NCH
        start = pl.multiple_of(c * T, T)
        return (
            pltpu.make_async_copy(k_hbm.at[0, h, pl.ds(start, T)], kbuf.at[slot],
                                  kv_sems.at[0, slot]),
            pltpu.make_async_copy(v_hbm.at[0, h, pl.ds(start, T)], vbuf.at[slot],
                                  kv_sems.at[1, slot]),
        )

    x_cp = pltpu.make_async_copy(x_hbm, xbuf, w_sems.at[0])
    wr_cp = pltpu.make_async_copy(wr_hbm, wrbuf, w_sems.at[1])
    wq_cp = pltpu.make_async_copy(wq_hbm, wqbuf, w_sems.at[2])
    wo_cp = pltpu.make_async_copy(wot_hbm, wobuf, w_sems.at[3])
    wg_cp = pltpu.make_async_copy(wg_hbm, wgbuf, w_sems.at[4])
    wu_cp = pltpu.make_async_copy(wu_hbm, wubuf, w_sems.at[5])
    wd_cps = [
        pltpu.make_async_copy(wdt_hbm.at[:, pl.ds(j * WD_PIECE, WD_PIECE)],
                              wdbuf.at[j], wd_sems.at[j])
        for j in range(N_WD)
    ]

    x_cp.start()
    wr_cp.start()
    wq_cp.start()
    for i in range(NBUF - 1):
        for cp in kv_copies(i, i):
            cp.start()
    wo_cp.start()

    x_cp.wait()
    x = xbuf[0].astype(f32)
    mean = jnp.mean(x, axis=-1, keepdims=True)
    xc = x - mean
    var = jnp.mean(xc * xc, axis=-1, keepdims=True)
    xn = xc / jnp.sqrt(var + EPS)
    xn_rows = jnp.broadcast_to(xn, (ROWS, D)).astype(bf16)

    row = lax.broadcasted_iota(jnp.int32, (ROWS, DH), 0)
    wq_cp.wait()
    for h in range(HKV):
        y = jnp.dot(xn_rows, wqbuf[:, h * REP * DH:(h + 1) * REP * DH],
                    preferred_element_type=f32)
        q_h = jnp.where(row == 0, y[:, :DH],
                        jnp.where(row == 1, y[:, DH:], 0.0))
        q_scr[h] = q_h.astype(bf16)

    scale = DH ** -0.5

    def body(i, carry):
        slot = i % NBUF
        h = i // NCH
        c = i % NCH
        nxt = i + NBUF - 1

        @pl.when(nxt < TOTAL)
        def _():
            for cp in kv_copies(nxt, nxt % NBUF):
                cp.start()

        @pl.when(nxt == TOTAL - 1)
        def _():
            wg_cp.start()
            wu_cp.start()
            for cp in wd_cps:
                cp.start()

        @pl.when(c == 0)
        def _():
            m_scr[...] = jnp.full(m_scr.shape, -jnp.inf, f32)
            l_scr[...] = jnp.zeros(l_scr.shape, f32)
            acc_scr[...] = jnp.zeros(acc_scr.shape, f32)

        k_cp, v_cp = kv_copies(i, slot)
        q = q_scr[h]
        k_cp.wait()
        s = lax.dot_general(q, kbuf[slot], _NT, preferred_element_type=f32) * scale
        m_old = m_scr[...]
        m_new = jnp.maximum(m_old, jnp.max(s, axis=1, keepdims=True))
        alpha = jnp.exp(m_old - m_new)
        p = jnp.exp(s - m_new)
        l_scr[...] = alpha * l_scr[...] + jnp.sum(p, axis=1, keepdims=True)
        m_scr[...] = m_new
        v_cp.wait()
        pv = jnp.dot(p.astype(bf16), vbuf[slot], preferred_element_type=f32)
        acc_scr[...] = alpha * acc_scr[...] + pv

        @pl.when(c == NCH - 1)
        def _():
            o_scr[h] = acc_scr[...] / l_scr[...]

        return carry

    lax.fori_loop(0, TOTAL, body, 0)

    wo_cp.wait()
    attn = jnp.zeros((ROWS, D), f32)
    for h in range(HKV):
        o_h = o_scr[h]
        z = jnp.concatenate(
            [jnp.where(row == 0, o_h, 0.0), jnp.where(row == 1, o_h, 0.0)],
            axis=1).astype(bf16)
        attn = attn + lax.dot_general(
            z, wobuf[:, h * REP * DH:(h + 1) * REP * DH], _NT,
            preferred_element_type=f32)
    attn = jnp.sum(attn, axis=0, keepdims=True)

    wr_cp.wait()
    wr = wrbuf[...].astype(f32).reshape(1, D)
    r = jnp.sum(xn_rows[0:1].astype(f32) * wr, axis=-1, keepdims=True)
    gate = jax.nn.sigmoid(r)

    wg_cp.wait()
    g = jnp.dot(xn_rows, wgbuf[...], preferred_element_type=f32)
    wu_cp.wait()
    u = jnp.dot(xn_rows, wubuf[...], preferred_element_type=f32)
    hid = (g * jax.nn.sigmoid(g) * u).astype(bf16)
    y = jnp.zeros((ROWS, D), f32)
    for j in range(N_WD):
        wd_cps[j].wait()
        y = y + lax.dot_general(hid[:, j * WD_PIECE:(j + 1) * WD_PIECE], wdbuf[j],
                                _NT, preferred_element_type=f32)
    y = y[0:1] * gate

    out = x + attn + (xn + (xn * 0.0 + y))
    o_ref[0] = out.astype(o_ref.dtype)


@jax.jit
def pallas_parallel_sum__gqa_block_cached__moe_arch_mod__decode_kernel(
    A_x: jax.Array,
    A_k_cache: jax.Array,
    A_v_cache: jax.Array,
    A_wq: jax.Array,
    A_wo: jax.Array,
    B_x: jax.Array,
    B_w_r: jax.Array,
    B_w_gate: jax.Array,
    B_w_up: jax.Array,
    B_w_down: jax.Array,
):
    del B_x
    bf16 = jnp.bfloat16
    f32 = jnp.float32
    any_spec = pl.BlockSpec(memory_space=pl.ANY)
    scratch = [
        pltpu.VMEM((1, 1, D), bf16),
        pltpu.VMEM((D,), bf16),
        pltpu.VMEM((D, HQ * DH), bf16),
        pltpu.VMEM((D, HQ * DH), bf16),
        pltpu.VMEM((D, F), bf16),
        pltpu.VMEM((D, F), bf16),
        pltpu.VMEM((N_WD, D, WD_PIECE), bf16),
        pltpu.VMEM((NBUF, T, DH), bf16),
        pltpu.VMEM((NBUF, T, DH), bf16),
        pltpu.VMEM((HKV, ROWS, DH), bf16),
        pltpu.VMEM((HKV, ROWS, DH), f32),
        pltpu.VMEM((ROWS, 1), f32),
        pltpu.VMEM((ROWS, 1), f32),
        pltpu.VMEM((ROWS, DH), f32),
        pltpu.SemaphoreType.DMA((2, NBUF)),
        pltpu.SemaphoreType.DMA((6,)),
        pltpu.SemaphoreType.DMA((N_WD,)),
    ]
    return pl.pallas_call(
        _kernel,
        out_shape=jax.ShapeDtypeStruct((1, 1, D), bf16),
        in_specs=[any_spec] * 9,
        out_specs=pl.BlockSpec(memory_space=pltpu.VMEM),
        scratch_shapes=scratch,
        compiler_params=pltpu.CompilerParams(vmem_limit_bytes=64 * 1024 * 1024),
    )(A_x, A_k_cache, A_v_cache, A_wq, A_wo.T, B_w_r, B_w_gate, B_w_up, B_w_down.T)
```

```python
import functools

import jax
import jax.numpy as jnp
from jax import lax
import jax.experimental.pallas as pl
import jax.experimental.pallas.tpu as pltpu

D = 448
HQ = 16
HKV = 8
REP = HQ // HKV
SK = 65536
DH = 256
F = 1792
ROWS = 8
EPS = 1e-5

T = 2048
NBUF = 4
NCH = SK // T
TOTAL = HKV * NCH
WD_PIECE = 256
N_WD = F // WD_PIECE

_NT = (((1,), (1,)), ((), ()))


def _kernel(x_hbm, k_hbm, v_hbm, wq_hbm, wot_hbm, wr_hbm, wg_hbm, wu_hbm, wdt_hbm,
            o_ref,
            xbuf, wrbuf, wqbuf, wobuf, wgbuf, wubuf, wdbuf, kbuf, vbuf,
            q_scr, o_scr, m_scr, l_scr, acc_scr,
            kv_sems, w_sems, wd_sems):
    f32 = jnp.float32
    bf16 = jnp.bfloat16

    def kv_copies(i, slot):
        h = i // NCH
        c = i % NCH
        start = pl.multiple_of(c * T, T)
        return (
            pltpu.make_async_copy(k_hbm.at[0, h, pl.ds(start, T)], kbuf.at[slot],
                                  kv_sems.at[0, slot]),
            pltpu.make_async_copy(v_hbm.at[0, h, pl.ds(start, T)], vbuf.at[slot],
                                  kv_sems.at[1, slot]),
        )

    x_cp = pltpu.make_async_copy(x_hbm, xbuf, w_sems.at[0])
    wr_cp = pltpu.make_async_copy(wr_hbm, wrbuf, w_sems.at[1])
    wq_cp = pltpu.make_async_copy(wq_hbm, wqbuf, w_sems.at[2])
    wo_cp = pltpu.make_async_copy(wot_hbm, wobuf, w_sems.at[3])
    wg_cp = pltpu.make_async_copy(wg_hbm, wgbuf, w_sems.at[4])
    wu_cp = pltpu.make_async_copy(wu_hbm, wubuf, w_sems.at[5])

    def wd_copy(j, start):
        return pltpu.make_async_copy(wdt_hbm.at[:, pl.ds(start, WD_PIECE)],
                                     wdbuf.at[j], wd_sems.at[j])

    x_cp.start()
    wr_cp.start()
    wq_cp.start()
    for i in range(NBUF - 1):
        for cp in kv_copies(i, i):
            cp.start()
    wo_cp.start()

    x_cp.wait()
    x = xbuf[0].astype(f32)
    mean = jnp.mean(x, axis=-1, keepdims=True)
    xc = x - mean
    var = jnp.mean(xc * xc, axis=-1, keepdims=True)
    xn = xc / jnp.sqrt(var + EPS)
    xn_rows = jnp.broadcast_to(xn, (ROWS, D)).astype(bf16)

    row = lax.broadcasted_iota(jnp.int32, (ROWS, DH), 0)
    wq_cp.wait()
    for h in range(HKV):
        y = jnp.dot(xn_rows, wqbuf[:, h * REP * DH:(h + 1) * REP * DH],
                    preferred_element_type=f32)
        q_h = jnp.where(row == 0, y[:, :DH],
                        jnp.where(row == 1, y[:, DH:], 0.0))
        q_scr[h] = q_h.astype(bf16)

    scale = DH ** -0.5

    def body(i, carry):
        slot = i % NBUF
        h = i // NCH
        c = i % NCH
        nxt = i + NBUF - 1

        @pl.when(nxt < TOTAL)
        def _():
            for cp in kv_copies(nxt, nxt % NBUF):
                cp.start()

        @pl.when(nxt == TOTAL)
        def _():
            wg_cp.start()

        @pl.when(nxt == TOTAL + 1)
        def _():
            wu_cp.start()

        @pl.when(nxt == TOTAL + 2)
        def _():
            def issue(j, c2):
                wd_copy(j, pl.multiple_of(j * WD_PIECE, WD_PIECE)).start()
                return c2
            lax.fori_loop(0, N_WD, issue, 0)

        @pl.when(c == 0)
        def _():
            m_scr[...] = jnp.full(m_scr.shape, -jnp.inf, f32)
            l_scr[...] = jnp.zeros(l_scr.shape, f32)
            acc_scr[...] = jnp.zeros(acc_scr.shape, f32)

        k_cp, v_cp = kv_copies(i, slot)
        q = q_scr[h]
        k_cp.wait()
        s = lax.dot_general(q, kbuf[slot], _NT, preferred_element_type=f32) * scale
        m_old = m_scr[...]
        m_new = jnp.maximum(m_old, jnp.max(s, axis=1, keepdims=True))
        alpha = jnp.exp(m_old - m_new)
        p = jnp.exp(s - m_new)
        l_scr[...] = alpha * l_scr[...] + jnp.sum(p, axis=1, keepdims=True)
        m_scr[...] = m_new
        v_cp.wait()
        pv = jnp.dot(p.astype(bf16), vbuf[slot], preferred_element_type=f32)
        acc_scr[...] = alpha * acc_scr[...] + pv

        @pl.when(c == NCH - 1)
        def _():
            o_scr[h] = acc_scr[...] / l_scr[...]

        return carry

    lax.fori_loop(0, TOTAL, body, 0)

    wo_cp.wait()
    attn = jnp.zeros((ROWS, D), f32)
    for h in range(HKV):
        o_h = o_scr[h]
        z = jnp.concatenate(
            [jnp.where(row == 0, o_h, 0.0), jnp.where(row == 1, o_h, 0.0)],
            axis=1).astype(bf16)
        attn = attn + lax.dot_general(
            z, wobuf[:, h * REP * DH:(h + 1) * REP * DH], _NT,
            preferred_element_type=f32)
    attn = jnp.sum(attn, axis=0, keepdims=True)

    wr_cp.wait()
    wr = wrbuf[...].astype(f32).reshape(1, D)
    r = jnp.sum(xn_rows[0:1].astype(f32) * wr, axis=-1, keepdims=True)
    gate = jax.nn.sigmoid(r)

    wg_cp.wait()
    g = jnp.dot(xn_rows, wgbuf[...], preferred_element_type=f32)
    wu_cp.wait()
    u = jnp.dot(xn_rows, wubuf[...], preferred_element_type=f32)
    hid = (g * jax.nn.sigmoid(g) * u).astype(bf16)
    y = jnp.zeros((ROWS, D), f32)
    for j in range(N_WD):
        wd_copy(j, j * WD_PIECE).wait()
        y = y + lax.dot_general(hid[:, j * WD_PIECE:(j + 1) * WD_PIECE], wdbuf[j],
                                _NT, preferred_element_type=f32)
    y = y[0:1] * gate

    out = x + attn + (xn + (xn * 0.0 + y))
    o_ref[0] = out.astype(o_ref.dtype)


@jax.jit
def pallas_parallel_sum__gqa_block_cached__moe_arch_mod__decode_kernel(
    A_x: jax.Array,
    A_k_cache: jax.Array,
    A_v_cache: jax.Array,
    A_wq: jax.Array,
    A_wo: jax.Array,
    B_x: jax.Array,
    B_w_r: jax.Array,
    B_w_gate: jax.Array,
    B_w_up: jax.Array,
    B_w_down: jax.Array,
):
    del B_x
    bf16 = jnp.bfloat16
    f32 = jnp.float32
    any_spec = pl.BlockSpec(memory_space=pl.ANY)
    scratch = [
        pltpu.VMEM((1, 1, D), bf16),
        pltpu.VMEM((D,), bf16),
        pltpu.VMEM((D, HQ * DH), bf16),
        pltpu.VMEM((D, HQ * DH), bf16),
        pltpu.VMEM((D, F), bf16),
        pltpu.VMEM((D, F), bf16),
        pltpu.VMEM((N_WD, D, WD_PIECE), bf16),
        pltpu.VMEM((NBUF, T, DH), bf16),
        pltpu.VMEM((NBUF, T, DH), bf16),
        pltpu.VMEM((HKV, ROWS, DH), bf16),
        pltpu.VMEM((HKV, ROWS, DH), f32),
        pltpu.VMEM((ROWS, 1), f32),
        pltpu.VMEM((ROWS, 1), f32),
        pltpu.VMEM((ROWS, DH), f32),
        pltpu.SemaphoreType.DMA((2, NBUF)),
        pltpu.SemaphoreType.DMA((6,)),
        pltpu.SemaphoreType.DMA((N_WD,)),
    ]
    return pl.pallas_call(
        _kernel,
        out_shape=jax.ShapeDtypeStruct((1, 1, D), bf16),
        in_specs=[any_spec] * 9,
        out_specs=pl.BlockSpec(memory_space=pltpu.VMEM),
        scratch_shapes=scratch,
        compiler_params=pltpu.CompilerParams(vmem_limit_bytes=64 * 1024 * 1024),
    )(A_x, A_k_cache, A_v_cache, A_wq, A_wo.T, B_w_r, B_w_gate, B_w_up, B_w_down.T)
```

```python
import functools

import jax
import jax.numpy as jnp
from jax import lax
import jax.experimental.pallas as pl
import jax.experimental.pallas.tpu as pltpu

D = 448
HQ = 16
HKV = 8
REP = HQ // HKV
SK = 65536
DH = 256
F = 1792
ROWS = 8
EPS = 1e-5

T = 2048
NBUF = 4
TP = 64
NCH = SK // T
TOTAL = HKV * NCH
WD_PIECE = 256
N_WD = F // WD_PIECE

_NT = (((1,), (1,)), ((), ()))


def _kernel(x_hbm, k_hbm, v_hbm, wq_hbm, wot_hbm, wr_hbm, wg_hbm, wu_hbm, wdt_hbm,
            o_ref,
            xbuf, wrbuf, wqbuf, wobuf, wgbuf, wubuf, wdbuf, kbuf, vbuf,
            q_scr, o_scr, m_scr, l_scr, acc_scr,
            kv_sems, w_sems, wd_sems):
    f32 = jnp.float32
    bf16 = jnp.bfloat16

    def kv_start(i, slot):
        h = i // NCH
        base = (i % NCH) * T

        def piece(j, c2):
            off = pl.multiple_of(j * TP, TP)
            src = pl.multiple_of(base + off, TP)
            pltpu.make_async_copy(k_hbm.at[0, h, pl.ds(src, TP)],
                                  kbuf.at[slot, pl.ds(off, TP)],
                                  kv_sems.at[0, slot]).start(priority=0)
            pltpu.make_async_copy(v_hbm.at[0, h, pl.ds(src, TP)],
                                  vbuf.at[slot, pl.ds(off, TP)],
                                  kv_sems.at[1, slot]).start(priority=1)
            return c2

        lax.fori_loop(0, T // TP, piece, 0, unroll=4)

    def k_wait(slot):
        pltpu.make_async_copy(kbuf.at[slot], kbuf.at[slot], kv_sems.at[0, slot]).wait()

    def v_wait(slot):
        pltpu.make_async_copy(vbuf.at[slot], vbuf.at[slot], kv_sems.at[1, slot]).wait()

    x_cp = pltpu.make_async_copy(x_hbm, xbuf, w_sems.at[0])
    wr_cp = pltpu.make_async_copy(wr_hbm, wrbuf, w_sems.at[1])
    wq_cp = pltpu.make_async_copy(wq_hbm, wqbuf, w_sems.at[2])
    wo_cp = pltpu.make_async_copy(wot_hbm, wobuf, w_sems.at[3])
    wg_cp = pltpu.make_async_copy(wg_hbm, wgbuf, w_sems.at[4])
    wu_cp = pltpu.make_async_copy(wu_hbm, wubuf, w_sems.at[5])

    def wd_copy(j, start):
        return pltpu.make_async_copy(wdt_hbm.at[:, pl.ds(start, WD_PIECE)],
                                     wdbuf.at[j], wd_sems.at[j])

    x_cp.start()
    wr_cp.start()
    wq_cp.start()
    for i in range(NBUF - 1):
        kv_start(i, i)
    wo_cp.start()

    x_cp.wait()
    x = xbuf[0].astype(f32)
    mean = jnp.mean(x, axis=-1, keepdims=True)
    xc = x - mean
    var = jnp.mean(xc * xc, axis=-1, keepdims=True)
    xn = xc / jnp.sqrt(var + EPS)
    xn_rows = jnp.broadcast_to(xn, (ROWS, D)).astype(bf16)

    row = lax.broadcasted_iota(jnp.int32, (ROWS, DH), 0)
    wq_cp.wait()
    for h in range(HKV):
        y = jnp.dot(xn_rows, wqbuf[:, h * REP * DH:(h + 1) * REP * DH],
                    preferred_element_type=f32)
        q_h = jnp.where(row == 0, y[:, :DH],
                        jnp.where(row == 1, y[:, DH:], 0.0))
        q_scr[h] = q_h.astype(bf16)

    scale = DH ** -0.5

    def body(i, carry):
        slot = i % NBUF
        h = i // NCH
        c = i % NCH
        nxt = i + NBUF - 1

        @pl.when(nxt < TOTAL)
        def _():
            kv_start(nxt, nxt % NBUF)

        @pl.when(nxt == TOTAL)
        def _():
            wg_cp.start()

        @pl.when(nxt == TOTAL + 1)
        def _():
            wu_cp.start()

        @pl.when(nxt == TOTAL + 2)
        def _():
            def issue(j, c2):
                wd_copy(j, pl.multiple_of(j * WD_PIECE, WD_PIECE)).start()
                return c2
            lax.fori_loop(0, N_WD, issue, 0)

        @pl.when(c == 0)
        def _():
            m_scr[...] = jnp.full(m_scr.shape, -jnp.inf, f32)
            l_scr[...] = jnp.zeros(l_scr.shape, f32)
            acc_scr[...] = jnp.zeros(acc_scr.shape, f32)

        q = q_scr[h]
        k_wait(slot)
        s = lax.dot_general(q, kbuf[slot], _NT, preferred_element_type=f32) * scale
        m_old = m_scr[...]
        m_new = jnp.maximum(m_old, jnp.max(s, axis=1, keepdims=True))
        alpha = jnp.exp(m_old - m_new)
        p = jnp.exp(s - m_new)
        l_scr[...] = alpha * l_scr[...] + jnp.sum(p, axis=1, keepdims=True)
        m_scr[...] = m_new
        v_wait(slot)
        pv = jnp.dot(p.astype(bf16), vbuf[slot], preferred_element_type=f32)
        acc_scr[...] = alpha * acc_scr[...] + pv

        @pl.when(c == NCH - 1)
        def _():
            o_scr[h] = acc_scr[...] / l_scr[...]

        return carry

    lax.fori_loop(0, TOTAL, body, 0)

    wo_cp.wait()
    attn = jnp.zeros((ROWS, D), f32)
    for h in range(HKV):
        o_h = o_scr[h]
        z = jnp.concatenate(
            [jnp.where(row == 0, o_h, 0.0), jnp.where(row == 1, o_h, 0.0)],
            axis=1).astype(bf16)
        attn = attn + lax.dot_general(
            z, wobuf[:, h * REP * DH:(h + 1) * REP * DH], _NT,
            preferred_element_type=f32)
    attn = jnp.sum(attn, axis=0, keepdims=True)

    wr_cp.wait()
    wr = wrbuf[...].astype(f32).reshape(1, D)
    r = jnp.sum(xn_rows[0:1].astype(f32) * wr, axis=-1, keepdims=True)
    gate = jax.nn.sigmoid(r)

    wg_cp.wait()
    g = jnp.dot(xn_rows, wgbuf[...], preferred_element_type=f32)
    wu_cp.wait()
    u = jnp.dot(xn_rows, wubuf[...], preferred_element_type=f32)
    hid = (g * jax.nn.sigmoid(g) * u).astype(bf16)
    y = jnp.zeros((ROWS, D), f32)
    for j in range(N_WD):
        wd_copy(j, j * WD_PIECE).wait()
        y = y + lax.dot_general(hid[:, j * WD_PIECE:(j + 1) * WD_PIECE], wdbuf[j],
                                _NT, preferred_element_type=f32)
    y = y[0:1] * gate

    out = x + attn + (xn + (xn * 0.0 + y))
    o_ref[0] = out.astype(o_ref.dtype)


@jax.jit
def pallas_parallel_sum__gqa_block_cached__moe_arch_mod__decode_kernel(
    A_x: jax.Array,
    A_k_cache: jax.Array,
    A_v_cache: jax.Array,
    A_wq: jax.Array,
    A_wo: jax.Array,
    B_x: jax.Array,
    B_w_r: jax.Array,
    B_w_gate: jax.Array,
    B_w_up: jax.Array,
    B_w_down: jax.Array,
):
    del B_x
    bf16 = jnp.bfloat16
    f32 = jnp.float32
    any_spec = pl.BlockSpec(memory_space=pl.ANY)
    scratch = [
        pltpu.VMEM((1, 1, D), bf16),
        pltpu.VMEM((D,), bf16),
        pltpu.VMEM((D, HQ * DH), bf16),
        pltpu.VMEM((D, HQ * DH), bf16),
        pltpu.VMEM((D, F), bf16),
        pltpu.VMEM((D, F), bf16),
        pltpu.VMEM((N_WD, D, WD_PIECE), bf16),
        pltpu.VMEM((NBUF, T, DH), bf16),
        pltpu.VMEM((NBUF, T, DH), bf16),
        pltpu.VMEM((HKV, ROWS, DH), bf16),
        pltpu.VMEM((HKV, ROWS, DH), f32),
        pltpu.VMEM((ROWS, 1), f32),
        pltpu.VMEM((ROWS, 1), f32),
        pltpu.VMEM((ROWS, DH), f32),
        pltpu.SemaphoreType.DMA((2, NBUF)),
        pltpu.SemaphoreType.DMA((6,)),
        pltpu.SemaphoreType.DMA((N_WD,)),
    ]
    return pl.pallas_call(
        _kernel,
        out_shape=jax.ShapeDtypeStruct((1, 1, D), bf16),
        in_specs=[any_spec] * 9,
        out_specs=pl.BlockSpec(memory_space=pltpu.VMEM),
        scratch_shapes=scratch,
        compiler_params=pltpu.CompilerParams(vmem_limit_bytes=64 * 1024 * 1024),
    )(A_x, A_k_cache, A_v_cache, A_wq, A_wo.T, B_w_r, B_w_gate, B_w_up, B_w_down.T)
```

```python
import functools

import jax
import jax.numpy as jnp
from jax import lax
import jax.experimental.pallas as pl
import jax.experimental.pallas.tpu as pltpu

D = 448
HQ = 16
HKV = 8
REP = HQ // HKV
SK = 65536
DH = 256
F = 1792
ROWS = 8
EPS = 1e-5

T = 2048
NBUF = 4
TP = 64
NCH = SK // T
TOTAL = HKV * NCH
assert NBUF >= 4
WD_PIECE = 256
N_WD = F // WD_PIECE

_NT = (((1,), (1,)), ((), ()))


def _kernel(x_hbm, k_hbm, v_hbm, wq_hbm, wot_hbm, wr_hbm, wg_hbm, wu_hbm, wdt_hbm,
            o_ref,
            xbuf, wrbuf, wqbuf, wobuf, wgbuf, wubuf, wdbuf, kbuf, vbuf,
            q_scr, o_scr, m_scr, l_scr, acc_scr,
            kv_sems, w_sems, wd_sems):
    f32 = jnp.float32
    bf16 = jnp.bfloat16

    def kv_start(i, slot):
        h = i // NCH
        base = (i % NCH) * T

        def piece(j, c2):
            off = pl.multiple_of(j * TP, TP)
            src = pl.multiple_of(base + off, TP)
            pltpu.make_async_copy(k_hbm.at[0, h, pl.ds(src, TP)],
                                  kbuf.at[slot, pl.ds(off, TP)],
                                  kv_sems.at[0, slot]).start(priority=0)
            pltpu.make_async_copy(v_hbm.at[0, h, pl.ds(src, TP)],
                                  vbuf.at[slot, pl.ds(off, TP)],
                                  kv_sems.at[1, slot]).start(priority=1)
            return c2

        lax.fori_loop(0, T // TP, piece, 0, unroll=4)

    def k_wait(slot):
        pltpu.make_async_copy(kbuf.at[slot], kbuf.at[slot], kv_sems.at[0, slot]).wait()

    def v_wait(slot):
        pltpu.make_async_copy(vbuf.at[slot], vbuf.at[slot], kv_sems.at[1, slot]).wait()

    x_cp = pltpu.make_async_copy(x_hbm, xbuf, w_sems.at[0])
    wr_cp = pltpu.make_async_copy(wr_hbm, wrbuf, w_sems.at[1])
    wq_cp = pltpu.make_async_copy(wq_hbm, wqbuf, w_sems.at[2])
    wo_cp = pltpu.make_async_copy(wot_hbm, wobuf, w_sems.at[3])
    wg_cp = pltpu.make_async_copy(wg_hbm, wgbuf, w_sems.at[4])
    wu_cp = pltpu.make_async_copy(wu_hbm, wubuf, w_sems.at[5])

    def wd_copy(j, start):
        return pltpu.make_async_copy(wdt_hbm.at[:, pl.ds(start, WD_PIECE)],
                                     wdbuf.at[j], wd_sems.at[j])

    x_cp.start()
    wr_cp.start()
    wq_cp.start()
    for i in range(NBUF - 1):
        kv_start(i, i)
    wo_cp.start()

    x_cp.wait()
    x = xbuf[0].astype(f32)
    mean = jnp.mean(x, axis=-1, keepdims=True)
    xc = x - mean
    var = jnp.mean(xc * xc, axis=-1, keepdims=True)
    xn = xc / jnp.sqrt(var + EPS)
    xn_rows = jnp.broadcast_to(xn, (ROWS, D)).astype(bf16)

    row = lax.broadcasted_iota(jnp.int32, (ROWS, DH), 0)
    wq_cp.wait()
    for h in range(HKV):
        y = jnp.dot(xn_rows, wqbuf[:, h * REP * DH:(h + 1) * REP * DH],
                    preferred_element_type=f32)
        q_h = jnp.where(row == 0, y[:, :DH],
                        jnp.where(row == 1, y[:, DH:], 0.0))
        q_scr[h] = q_h.astype(bf16)

    scale = DH ** -0.5

    def body(i, carry):
        slot = i % NBUF
        h = i // NCH
        c = i % NCH
        nxt = i + NBUF - 1

        @pl.when(nxt < TOTAL)
        def _():
            kv_start(nxt, nxt % NBUF)

        @pl.when(nxt == TOTAL)
        def _():
            wg_cp.start(priority=1)

        @pl.when(nxt == TOTAL + 1)
        def _():
            wu_cp.start(priority=1)

        @pl.when(nxt == TOTAL + 2)
        def _():
            def issue(j, c2):
                wd_copy(j, pl.multiple_of(j * WD_PIECE, WD_PIECE)).start(priority=1)
                return c2
            lax.fori_loop(0, N_WD, issue, 0)

        @pl.when(c == 0)
        def _():
            m_scr[...] = jnp.full(m_scr.shape, -jnp.inf, f32)
            l_scr[...] = jnp.zeros(l_scr.shape, f32)
            acc_scr[...] = jnp.zeros(acc_scr.shape, f32)

        q = q_scr[h]
        k_wait(slot)
        s = lax.dot_general(q, kbuf[slot], _NT, preferred_element_type=f32) * scale
        m_old = m_scr[...]
        m_new = jnp.maximum(m_old, jnp.max(s, axis=1, keepdims=True))
        alpha = jnp.exp(m_old - m_new)
        p = jnp.exp(s - m_new)
        l_scr[...] = alpha * l_scr[...] + jnp.sum(p, axis=1, keepdims=True)
        m_scr[...] = m_new
        v_wait(slot)
        pv = jnp.dot(p.astype(bf16), vbuf[slot], preferred_element_type=f32)
        acc_scr[...] = alpha * acc_scr[...] + pv

        @pl.when(c == NCH - 1)
        def _():
            o_scr[h] = acc_scr[...] / l_scr[...]

        return carry

    lax.fori_loop(0, TOTAL, body, 0)

    wo_cp.wait()
    attn = jnp.zeros((ROWS, D), f32)
    for h in range(HKV):
        o_h = o_scr[h]
        z = jnp.concatenate(
            [jnp.where(row == 0, o_h, 0.0), jnp.where(row == 1, o_h, 0.0)],
            axis=1).astype(bf16)
        attn = attn + lax.dot_general(
            z, wobuf[:, h * REP * DH:(h + 1) * REP * DH], _NT,
            preferred_element_type=f32)
    attn = jnp.sum(attn, axis=0, keepdims=True)

    wr_cp.wait()
    wr = wrbuf[...].astype(f32).reshape(1, D)
    r = jnp.sum(xn_rows[0:1].astype(f32) * wr, axis=-1, keepdims=True)
    gate = jax.nn.sigmoid(r)

    wg_cp.wait()
    g = jnp.dot(xn_rows, wgbuf[...], preferred_element_type=f32)
    wu_cp.wait()
    u = jnp.dot(xn_rows, wubuf[...], preferred_element_type=f32)
    hid = (g * jax.nn.sigmoid(g) * u).astype(bf16)
    y = jnp.zeros((ROWS, D), f32)
    for j in range(N_WD):
        wd_copy(j, j * WD_PIECE).wait()
        y = y + lax.dot_general(hid[:, j * WD_PIECE:(j + 1) * WD_PIECE], wdbuf[j],
                                _NT, preferred_element_type=f32)
    y = y[0:1] * gate

    out = x + attn + (xn + (xn * 0.0 + y))
    o_ref[0] = out.astype(o_ref.dtype)


@jax.jit
def pallas_parallel_sum__gqa_block_cached__moe_arch_mod__decode_kernel(
    A_x: jax.Array,
    A_k_cache: jax.Array,
    A_v_cache: jax.Array,
    A_wq: jax.Array,
    A_wo: jax.Array,
    B_x: jax.Array,
    B_w_r: jax.Array,
    B_w_gate: jax.Array,
    B_w_up: jax.Array,
    B_w_down: jax.Array,
):
    del B_x
    bf16 = jnp.bfloat16
    f32 = jnp.float32
    any_spec = pl.BlockSpec(memory_space=pl.ANY)
    scratch = [
        pltpu.VMEM((1, 1, D), bf16),
        pltpu.VMEM((D,), bf16),
        pltpu.VMEM((D, HQ * DH), bf16),
        pltpu.VMEM((D, HQ * DH), bf16),
        pltpu.VMEM((D, F), bf16),
        pltpu.VMEM((D, F), bf16),
        pltpu.VMEM((N_WD, D, WD_PIECE), bf16),
        pltpu.VMEM((NBUF, T, DH), bf16),
        pltpu.VMEM((NBUF, T, DH), bf16),
        pltpu.VMEM((HKV, ROWS, DH), bf16),
        pltpu.VMEM((HKV, ROWS, DH), f32),
        pltpu.VMEM((ROWS, 1), f32),
        pltpu.VMEM((ROWS, 1), f32),
        pltpu.VMEM((ROWS, DH), f32),
        pltpu.SemaphoreType.DMA((2, NBUF)),
        pltpu.SemaphoreType.DMA((6,)),
        pltpu.SemaphoreType.DMA((N_WD,)),
    ]
    return pl.pallas_call(
        _kernel,
        out_shape=jax.ShapeDtypeStruct((1, 1, D), bf16),
        in_specs=[any_spec] * 9,
        out_specs=pl.BlockSpec(memory_space=pltpu.VMEM),
        scratch_shapes=scratch,
        compiler_params=pltpu.CompilerParams(vmem_limit_bytes=64 * 1024 * 1024),
    )(A_x, A_k_cache, A_v_cache, A_wq, A_wo.T, B_w_r, B_w_gate, B_w_up, B_w_down.T)
```

```python
import functools

import jax
import jax.numpy as jnp
from jax import lax
import jax.experimental.pallas as pl
import jax.experimental.pallas.tpu as pltpu

D = 448
HQ = 16
HKV = 8
REP = HQ // HKV
SK = 65536
DH = 256
F = 1792
ROWS = 8
EPS = 1e-5

T = 2048
NBUF = 4
TP = 64
NSEG = 4
SEG = SK // NSEG
PER = T // NSEG
NCH = SK // T
TOTAL = HKV * NCH
assert NBUF >= 4
WD_PIECE = 256
N_WD = F // WD_PIECE

_NT = (((1,), (1,)), ((), ()))


def _kernel(x_hbm, k_hbm, v_hbm, wq_hbm, wot_hbm, wr_hbm, wg_hbm, wu_hbm, wdt_hbm,
            o_ref,
            xbuf, wrbuf, wqbuf, wobuf, wgbuf, wubuf, wdbuf, kbuf, vbuf,
            q_scr, o_scr, m_scr, l_scr, acc_scr,
            kv_sems, w_sems, wd_sems):
    f32 = jnp.float32
    bf16 = jnp.bfloat16

    def kv_start(i, slot):
        h = i // NCH
        base = (i % NCH) * PER

        def piece(j, c2):
            for s in range(NSEG):
                off = pl.multiple_of(s * PER + j * TP, TP)
                src = pl.multiple_of(s * SEG + base + j * TP, TP)
                pltpu.make_async_copy(k_hbm.at[0, h, pl.ds(src, TP)],
                                      kbuf.at[slot, pl.ds(off, TP)],
                                      kv_sems.at[0, slot]).start(priority=0)
                pltpu.make_async_copy(v_hbm.at[0, h, pl.ds(src, TP)],
                                      vbuf.at[slot, pl.ds(off, TP)],
                                      kv_sems.at[1, slot]).start(priority=1)
            return c2

        lax.fori_loop(0, PER // TP, piece, 0)

    def k_wait(slot):
        pltpu.make_async_copy(kbuf.at[slot], kbuf.at[slot], kv_sems.at[0, slot]).wait()

    def v_wait(slot):
        pltpu.make_async_copy(vbuf.at[slot], vbuf.at[slot], kv_sems.at[1, slot]).wait()

    x_cp = pltpu.make_async_copy(x_hbm, xbuf, w_sems.at[0])
    wr_cp = pltpu.make_async_copy(wr_hbm, wrbuf, w_sems.at[1])
    wq_cp = pltpu.make_async_copy(wq_hbm, wqbuf, w_sems.at[2])
    wo_cp = pltpu.make_async_copy(wot_hbm, wobuf, w_sems.at[3])
    wg_cp = pltpu.make_async_copy(wg_hbm, wgbuf, w_sems.at[4])
    wu_cp = pltpu.make_async_copy(wu_hbm, wubuf, w_sems.at[5])

    def wd_copy(j, start):
        return pltpu.make_async_copy(wdt_hbm.at[:, pl.ds(start, WD_PIECE)],
                                     wdbuf.at[j], wd_sems.at[j])

    x_cp.start()
    wr_cp.start()
    wq_cp.start()
    for i in range(NBUF - 1):
        kv_start(i, i)
    wo_cp.start()

    x_cp.wait()
    x = xbuf[0].astype(f32)
    mean = jnp.mean(x, axis=-1, keepdims=True)
    xc = x - mean
    var = jnp.mean(xc * xc, axis=-1, keepdims=True)
    xn = xc / jnp.sqrt(var + EPS)
    xn_rows = jnp.broadcast_to(xn, (ROWS, D)).astype(bf16)

    row = lax.broadcasted_iota(jnp.int32, (ROWS, DH), 0)
    wq_cp.wait()
    for h in range(HKV):
        y = jnp.dot(xn_rows, wqbuf[:, h * REP * DH:(h + 1) * REP * DH],
                    preferred_element_type=f32)
        q_h = jnp.where(row == 0, y[:, :DH],
                        jnp.where(row == 1, y[:, DH:], 0.0))
        q_scr[h] = q_h.astype(bf16)

    scale = DH ** -0.5

    def body(i, carry):
        slot = i % NBUF
        h = i // NCH
        c = i % NCH
        nxt = i + NBUF - 1

        @pl.when(nxt < TOTAL)
        def _():
            kv_start(nxt, nxt % NBUF)

        @pl.when(nxt == TOTAL)
        def _():
            wg_cp.start(priority=1)

        @pl.when(nxt == TOTAL + 1)
        def _():
            wu_cp.start(priority=1)

        @pl.when(nxt == TOTAL + 2)
        def _():
            def issue(j, c2):
                wd_copy(j, pl.multiple_of(j * WD_PIECE, WD_PIECE)).start(priority=1)
                return c2
            lax.fori_loop(0, N_WD, issue, 0)

        @pl.when(c == 0)
        def _():
            m_scr[...] = jnp.full(m_scr.shape, -jnp.inf, f32)
            l_scr[...] = jnp.zeros(l_scr.shape, f32)
            acc_scr[...] = jnp.zeros(acc_scr.shape, f32)

        q = q_scr[h]
        k_wait(slot)
        s = lax.dot_general(q, kbuf[slot], _NT, preferred_element_type=f32) * scale
        m_old = m_scr[...]
        m_new = jnp.maximum(m_old, jnp.max(s, axis=1, keepdims=True))
        alpha = jnp.exp(m_old - m_new)
        p = jnp.exp(s - m_new)
        l_scr[...] = alpha * l_scr[...] + jnp.sum(p, axis=1, keepdims=True)
        m_scr[...] = m_new
        v_wait(slot)
        pv = jnp.dot(p.astype(bf16), vbuf[slot], preferred_element_type=f32)
        acc_scr[...] = alpha * acc_scr[...] + pv

        @pl.when(c == NCH - 1)
        def _():
            o_scr[h] = acc_scr[...] / l_scr[...]

        return carry

    lax.fori_loop(0, TOTAL, body, 0)

    wo_cp.wait()
    attn = jnp.zeros((ROWS, D), f32)
    for h in range(HKV):
        o_h = o_scr[h]
        z = jnp.concatenate(
            [jnp.where(row == 0, o_h, 0.0), jnp.where(row == 1, o_h, 0.0)],
            axis=1).astype(bf16)
        attn = attn + lax.dot_general(
            z, wobuf[:, h * REP * DH:(h + 1) * REP * DH], _NT,
            preferred_element_type=f32)
    attn = jnp.sum(attn, axis=0, keepdims=True)

    wr_cp.wait()
    wr = wrbuf[...].astype(f32).reshape(1, D)
    r = jnp.sum(xn_rows[0:1].astype(f32) * wr, axis=-1, keepdims=True)
    gate = jax.nn.sigmoid(r)

    wg_cp.wait()
    g = jnp.dot(xn_rows, wgbuf[...], preferred_element_type=f32)
    wu_cp.wait()
    u = jnp.dot(xn_rows, wubuf[...], preferred_element_type=f32)
    hid = (g * jax.nn.sigmoid(g) * u).astype(bf16)
    y = jnp.zeros((ROWS, D), f32)
    for j in range(N_WD):
        wd_copy(j, j * WD_PIECE).wait()
        y = y + lax.dot_general(hid[:, j * WD_PIECE:(j + 1) * WD_PIECE], wdbuf[j],
                                _NT, preferred_element_type=f32)
    y = y[0:1] * gate

    out = x + attn + (xn + (xn * 0.0 + y))
    o_ref[0] = out.astype(o_ref.dtype)


@jax.jit
def pallas_parallel_sum__gqa_block_cached__moe_arch_mod__decode_kernel(
    A_x: jax.Array,
    A_k_cache: jax.Array,
    A_v_cache: jax.Array,
    A_wq: jax.Array,
    A_wo: jax.Array,
    B_x: jax.Array,
    B_w_r: jax.Array,
    B_w_gate: jax.Array,
    B_w_up: jax.Array,
    B_w_down: jax.Array,
):
    del B_x
    bf16 = jnp.bfloat16
    f32 = jnp.float32
    any_spec = pl.BlockSpec(memory_space=pl.ANY)
    scratch = [
        pltpu.VMEM((1, 1, D), bf16),
        pltpu.VMEM((D,), bf16),
        pltpu.VMEM((D, HQ * DH), bf16),
        pltpu.VMEM((D, HQ * DH), bf16),
        pltpu.VMEM((D, F), bf16),
        pltpu.VMEM((D, F), bf16),
        pltpu.VMEM((N_WD, D, WD_PIECE), bf16),
        pltpu.VMEM((NBUF, T, DH), bf16),
        pltpu.VMEM((NBUF, T, DH), bf16),
        pltpu.VMEM((HKV, ROWS, DH), bf16),
        pltpu.VMEM((HKV, ROWS, DH), f32),
        pltpu.VMEM((ROWS, 1), f32),
        pltpu.VMEM((ROWS, 1), f32),
        pltpu.VMEM((ROWS, DH), f32),
        pltpu.SemaphoreType.DMA((2, NBUF)),
        pltpu.SemaphoreType.DMA((6,)),
        pltpu.SemaphoreType.DMA((N_WD,)),
    ]
    return pl.pallas_call(
        _kernel,
        out_shape=jax.ShapeDtypeStruct((1, 1, D), bf16),
        in_specs=[any_spec] * 9,
        out_specs=pl.BlockSpec(memory_space=pltpu.VMEM),
        scratch_shapes=scratch,
        compiler_params=pltpu.CompilerParams(vmem_limit_bytes=64 * 1024 * 1024),
    )(A_x, A_k_cache, A_v_cache, A_wq, A_wo.T, B_w_r, B_w_gate, B_w_up, B_w_down.T)
```

```python
import functools

import jax
import jax.numpy as jnp
from jax import lax
import jax.experimental.pallas as pl
import jax.experimental.pallas.tpu as pltpu

D = 448
HQ = 16
HKV = 8
REP = HQ // HKV
SK = 65536
DH = 256
F = 1792
ROWS = 8
EPS = 1e-5

T = 2048
NBUF = 4
TP = 64
NSEG = 4
SEG = SK // NSEG
PER = T // NSEG
NCH = SK // T
TOTAL = HKV * NCH
assert NBUF >= 4
WD_PIECE = 256
N_WD = F // WD_PIECE

_NT = (((1,), (1,)), ((), ()))


def _kernel(x_hbm, k_hbm, v_hbm, wq_hbm, wot_hbm, wr_hbm, wg_hbm, wu_hbm, wdt_hbm,
            o_ref,
            xbuf, wrbuf, wqbuf, wobuf, wgbuf, wubuf, wdbuf, kbuf, vbuf,
            q_scr, o_scr, m_scr, l_scr, acc_scr,
            kv_sems, w_sems, wd_sems):
    f32 = jnp.float32
    bf16 = jnp.bfloat16

    def kv_start(i, slot):
        h = i // NCH
        base = (i % NCH) * PER

        def piece(j, c2):
            for s in range(NSEG):
                off = pl.multiple_of(s * PER + j * TP, TP)
                src = pl.multiple_of(s * SEG + base + j * TP, TP)
                pltpu.make_async_copy(k_hbm.at[0, h, pl.ds(src, TP)],
                                      kbuf.at[slot, pl.ds(off, TP)],
                                      kv_sems.at[0, slot]).start(priority=0)
                pltpu.make_async_copy(v_hbm.at[0, h, pl.ds(src, TP)],
                                      vbuf.at[slot, pl.ds(off, TP)],
                                      kv_sems.at[1, slot]).start(priority=1)
            return c2

        lax.fori_loop(0, PER // TP, piece, 0)

    def k_wait(slot):
        pltpu.make_async_copy(kbuf.at[slot], kbuf.at[slot], kv_sems.at[0, slot]).wait()

    def v_wait(slot):
        pltpu.make_async_copy(vbuf.at[slot], vbuf.at[slot], kv_sems.at[1, slot]).wait()

    x_cp = pltpu.make_async_copy(x_hbm, xbuf, w_sems.at[0])
    wr_cp = pltpu.make_async_copy(wr_hbm, wrbuf, w_sems.at[1])

    def wqo_start():
        def piece(j, c2):
            lane = pl.multiple_of((j % 2) * (HQ * DH // 2), 128)
            for half in range(2):
                r = pl.multiple_of(half * (D // 2) + (j // 2) * 8, 8)
                idx = (pl.ds(r, 8), pl.ds(lane, HQ * DH // 2))
                pltpu.make_async_copy(wq_hbm.at[idx], wqbuf.at[idx],
                                      w_sems.at[2]).start(priority=0)
                pltpu.make_async_copy(wot_hbm.at[idx], wobuf.at[idx],
                                      w_sems.at[3]).start(priority=1)
            return c2

        lax.fori_loop(0, 2 * (D // 2 // 8), piece, 0)

    wq_cp = pltpu.make_async_copy(wqbuf, wqbuf, w_sems.at[2])
    wo_cp = pltpu.make_async_copy(wobuf, wobuf, w_sems.at[3])
    wg_cp = pltpu.make_async_copy(wg_hbm, wgbuf, w_sems.at[4])
    wu_cp = pltpu.make_async_copy(wu_hbm, wubuf, w_sems.at[5])

    def wd_copy(j, start):
        return pltpu.make_async_copy(wdt_hbm.at[:, pl.ds(start, WD_PIECE)],
                                     wdbuf.at[j], wd_sems.at[j])

    x_cp.start()
    wr_cp.start()
    wqo_start()
    for i in range(NBUF - 1):
        kv_start(i, i)

    x_cp.wait()
    x = xbuf[0].astype(f32)
    mean = jnp.mean(x, axis=-1, keepdims=True)
    xc = x - mean
    var = jnp.mean(xc * xc, axis=-1, keepdims=True)
    xn = xc / jnp.sqrt(var + EPS)
    xn_rows = jnp.broadcast_to(xn, (ROWS, D)).astype(bf16)

    row = lax.broadcasted_iota(jnp.int32, (ROWS, DH), 0)
    wq_cp.wait()
    for h in range(HKV):
        y = jnp.dot(xn_rows, wqbuf[:, h * REP * DH:(h + 1) * REP * DH],
                    preferred_element_type=f32)
        q_h = jnp.where(row == 0, y[:, :DH],
                        jnp.where(row == 1, y[:, DH:], 0.0))
        q_scr[h] = q_h.astype(bf16)

    scale = DH ** -0.5

    def body(i, carry):
        slot = i % NBUF
        h = i // NCH
        c = i % NCH
        nxt = i + NBUF - 1

        @pl.when(nxt < TOTAL)
        def _():
            kv_start(nxt, nxt % NBUF)

        @pl.when(nxt == TOTAL)
        def _():
            wg_cp.start(priority=1)

        @pl.when(nxt == TOTAL + 1)
        def _():
            wu_cp.start(priority=1)

        @pl.when(nxt == TOTAL + 2)
        def _():
            def issue(j, c2):
                wd_copy(j, pl.multiple_of(j * WD_PIECE, WD_PIECE)).start(priority=1)
                return c2
            lax.fori_loop(0, N_WD, issue, 0)

        @pl.when(c == 0)
        def _():
            m_scr[...] = jnp.full(m_scr.shape, -jnp.inf, f32)
            l_scr[...] = jnp.zeros(l_scr.shape, f32)
            acc_scr[...] = jnp.zeros(acc_scr.shape, f32)

        q = q_scr[h]
        k_wait(slot)
        s = lax.dot_general(q, kbuf[slot], _NT, preferred_element_type=f32) * scale
        m_old = m_scr[...]
        m_new = jnp.maximum(m_old, jnp.max(s, axis=1, keepdims=True))
        alpha = jnp.exp(m_old - m_new)
        p = jnp.exp(s - m_new)
        l_scr[...] = alpha * l_scr[...] + jnp.sum(p, axis=1, keepdims=True)
        m_scr[...] = m_new
        v_wait(slot)
        pv = jnp.dot(p.astype(bf16), vbuf[slot], preferred_element_type=f32)
        acc_scr[...] = alpha * acc_scr[...] + pv

        @pl.when(c == NCH - 1)
        def _():
            o_scr[h] = acc_scr[...] / l_scr[...]

        return carry

    lax.fori_loop(0, TOTAL, body, 0)

    wo_cp.wait()
    attn = jnp.zeros((ROWS, D), f32)
    for h in range(HKV):
        o_h = o_scr[h]
        z = jnp.concatenate(
            [jnp.where(row == 0, o_h, 0.0), jnp.where(row == 1, o_h, 0.0)],
            axis=1).astype(bf16)
        attn = attn + lax.dot_general(
            z, wobuf[:, h * REP * DH:(h + 1) * REP * DH], _NT,
            preferred_element_type=f32)
    attn = jnp.sum(attn, axis=0, keepdims=True)

    wr_cp.wait()
    wr = wrbuf[...].astype(f32).reshape(1, D)
    r = jnp.sum(xn_rows[0:1].astype(f32) * wr, axis=-1, keepdims=True)
    gate = jax.nn.sigmoid(r)

    wg_cp.wait()
    g = jnp.dot(xn_rows, wgbuf[...], preferred_element_type=f32)
    wu_cp.wait()
    u = jnp.dot(xn_rows, wubuf[...], preferred_element_type=f32)
    hid = (g * jax.nn.sigmoid(g) * u).astype(bf16)
    y = jnp.zeros((ROWS, D), f32)
    for j in range(N_WD):
        wd_copy(j, j * WD_PIECE).wait()
        y = y + lax.dot_general(hid[:, j * WD_PIECE:(j + 1) * WD_PIECE], wdbuf[j],
                                _NT, preferred_element_type=f32)
    y = y[0:1] * gate

    out = x + attn + (xn + (xn * 0.0 + y))
    o_ref[0] = out.astype(o_ref.dtype)


@jax.jit
def pallas_parallel_sum__gqa_block_cached__moe_arch_mod__decode_kernel(
    A_x: jax.Array,
    A_k_cache: jax.Array,
    A_v_cache: jax.Array,
    A_wq: jax.Array,
    A_wo: jax.Array,
    B_x: jax.Array,
    B_w_r: jax.Array,
    B_w_gate: jax.Array,
    B_w_up: jax.Array,
    B_w_down: jax.Array,
):
    del B_x
    bf16 = jnp.bfloat16
    f32 = jnp.float32
    any_spec = pl.BlockSpec(memory_space=pl.ANY)
    scratch = [
        pltpu.VMEM((1, 1, D), bf16),
        pltpu.VMEM((D,), bf16),
        pltpu.VMEM((D, HQ * DH), bf16),
        pltpu.VMEM((D, HQ * DH), bf16),
        pltpu.VMEM((D, F), bf16),
        pltpu.VMEM((D, F), bf16),
        pltpu.VMEM((N_WD, D, WD_PIECE), bf16),
        pltpu.VMEM((NBUF, T, DH), bf16),
        pltpu.VMEM((NBUF, T, DH), bf16),
        pltpu.VMEM((HKV, ROWS, DH), bf16),
        pltpu.VMEM((HKV, ROWS, DH), f32),
        pltpu.VMEM((ROWS, 1), f32),
        pltpu.VMEM((ROWS, 1), f32),
        pltpu.VMEM((ROWS, DH), f32),
        pltpu.SemaphoreType.DMA((2, NBUF)),
        pltpu.SemaphoreType.DMA((6,)),
        pltpu.SemaphoreType.DMA((N_WD,)),
    ]
    return pl.pallas_call(
        _kernel,
        out_shape=jax.ShapeDtypeStruct((1, 1, D), bf16),
        in_specs=[any_spec] * 9,
        out_specs=pl.BlockSpec(memory_space=pltpu.VMEM),
        scratch_shapes=scratch,
        compiler_params=pltpu.CompilerParams(vmem_limit_bytes=64 * 1024 * 1024),
    )(A_x, A_k_cache, A_v_cache, A_wq, A_wo.T, B_w_r, B_w_gate, B_w_up, B_w_down.T)
```

```python
import functools

import jax
import jax.numpy as jnp
from jax import lax
import jax.experimental.pallas as pl
import jax.experimental.pallas.tpu as pltpu

D = 448
HQ = 16
HKV = 8
REP = HQ // HKV
SK = 65536
DH = 256
F = 1792
ROWS = 8
EPS = 1e-5

T = 2048
NBUF = 4
NSEG = 8
TP = 8
SEG = SK // NSEG
PER = T // NSEG
NCH = SK // T
TOTAL = HKV * NCH
assert NBUF >= 2
WD_PIECE = 256
N_WD = F // WD_PIECE

_NT = (((1,), (1,)), ((), ()))


def _kernel(x_hbm, k_hbm, v_hbm, wq_hbm, wot_hbm, wr_hbm, wg_hbm, wu_hbm, wdt_hbm,
            o_ref,
            xbuf, wrbuf, wqbuf, wobuf, wgbuf, wubuf, wdbuf, kbuf, vbuf,
            q_scr, hid_scr, attn_scr, m_scr, l_scr, acc_scr,
            kv_sems, w_sems, wd_sems):
    f32 = jnp.float32
    bf16 = jnp.bfloat16

    def kv_start(i, slot):
        h = i // NCH
        base = (i % NCH) * PER

        def piece(j, c2):
            off = pl.multiple_of(j * TP, TP)
            src = pl.multiple_of(base + off, TP)
            pltpu.make_async_copy(v_hbm.at[h, :, pl.ds(src, TP)],
                                  vbuf.at[slot, :, pl.ds(off, TP)],
                                  kv_sems.at[1, slot]).start(priority=1)
            pltpu.make_async_copy(k_hbm.at[h, :, pl.ds(src, TP)],
                                  kbuf.at[slot, :, pl.ds(off, TP)],
                                  kv_sems.at[0, slot]).start(priority=0)
            return c2

        lax.fori_loop(0, PER // TP, piece, 0)

    def k_wait(slot):
        pltpu.make_async_copy(kbuf.at[slot], kbuf.at[slot], kv_sems.at[0, slot]).wait()

    def v_wait(slot):
        pltpu.make_async_copy(vbuf.at[slot], vbuf.at[slot], kv_sems.at[1, slot]).wait()

    x_cp = pltpu.make_async_copy(x_hbm, xbuf, w_sems.at[0])
    wr_cp = pltpu.make_async_copy(wr_hbm, wrbuf, w_sems.at[1])

    def wqo_start():
        def piece(j, c2):
            lane = pl.multiple_of((j % 2) * (HQ * DH // 2), 128)
            for half in range(2):
                r = pl.multiple_of(half * (D // 2) + (j // 2) * 8, 8)
                idx = (pl.ds(r, 8), pl.ds(lane, HQ * DH // 2))
                pltpu.make_async_copy(wq_hbm.at[idx], wqbuf.at[idx],
                                      w_sems.at[2]).start(priority=0)
                pltpu.make_async_copy(wot_hbm.at[idx], wobuf.at[idx],
                                      w_sems.at[3]).start(priority=1)
            return c2

        lax.fori_loop(0, 2 * (D // 2 // 8), piece, 0)

    wq_cp = pltpu.make_async_copy(wqbuf, wqbuf, w_sems.at[2])
    wo_cp = pltpu.make_async_copy(wobuf, wobuf, w_sems.at[3])

    def wgu_start():
        def piece(j, c2):
            for half in range(2):
                r = pl.multiple_of(half * (D // 2) + j * 8, 8)
                pltpu.make_async_copy(wg_hbm.at[pl.ds(r, 8)], wgbuf.at[pl.ds(r, 8)],
                                      w_sems.at[4]).start(priority=0)
                pltpu.make_async_copy(wu_hbm.at[pl.ds(r, 8)], wubuf.at[pl.ds(r, 8)],
                                      w_sems.at[5]).start(priority=1)
            return c2

        lax.fori_loop(0, D // 2 // 8, piece, 0)

    wg_cp = pltpu.make_async_copy(wgbuf, wgbuf, w_sems.at[4])
    wu_cp = pltpu.make_async_copy(wubuf, wubuf, w_sems.at[5])

    def wd_start():
        def group(g, c2):
            lane = pl.multiple_of(g * WD_PIECE, WD_PIECE)
            pltpu.make_async_copy(wdt_hbm.at[:, pl.ds(lane, WD_PIECE)], wdbuf.at[g],
                                  wd_sems.at[g]).start(priority=1)
            return c2

        lax.fori_loop(0, N_WD, group, 0)

    def wd_wait(g):
        pltpu.make_async_copy(wdbuf.at[g], wdbuf.at[g], wd_sems.at[g]).wait()

    x_cp.start()
    wr_cp.start()
    wqo_start()
    wgu_start()

    x_cp.wait()
    x = xbuf[0].astype(f32)
    mean = jnp.mean(x, axis=-1, keepdims=True)
    xc = x - mean
    var = jnp.mean(xc * xc, axis=-1, keepdims=True)
    xn = xc / jnp.sqrt(var + EPS)
    xn_rows = jnp.broadcast_to(xn, (ROWS, D)).astype(bf16)

    row = lax.broadcasted_iota(jnp.int32, (ROWS, DH), 0)
    wq_cp.wait()
    for h in range(HKV):
        y = jnp.dot(xn_rows, wqbuf[:, h * REP * DH:(h + 1) * REP * DH],
                    preferred_element_type=f32)
        q_h = jnp.where(row == 0, y[:, :DH],
                        jnp.where(row == 1, y[:, DH:], 0.0))
        q_scr[h] = q_h.astype(bf16)

    for i in range(NBUF - 1):
        kv_start(i, i)

    wr_cp.wait()
    wr = wrbuf[...].astype(f32).reshape(1, D)
    r = jnp.sum(xn_rows[0:1].astype(f32) * wr, axis=-1, keepdims=True)
    gate = jax.nn.sigmoid(r)
    wg_cp.wait()
    g = jnp.dot(xn_rows, wgbuf[...], preferred_element_type=f32)
    wu_cp.wait()
    u = jnp.dot(xn_rows, wubuf[...], preferred_element_type=f32)
    hid_scr[...] = (g * jax.nn.sigmoid(g) * u).astype(bf16)
    attn_scr[...] = jnp.zeros(attn_scr.shape, f32)
    wo_cp.wait()

    scale = DH ** -0.5

    def body(i, carry):
        slot = i % NBUF
        h = i // NCH
        c = i % NCH
        nxt = i + NBUF - 1

        @pl.when(nxt < TOTAL)
        def _():
            kv_start(nxt, nxt % NBUF)

        @pl.when(nxt == TOTAL)
        def _():
            wd_start()

        @pl.when(c == 0)
        def _():
            m_scr[...] = jnp.full(m_scr.shape, -jnp.inf, f32)
            l_scr[...] = jnp.zeros(l_scr.shape, f32)
            acc_scr[...] = jnp.zeros(acc_scr.shape, f32)

        q = q_scr[h]
        k_wait(slot)
        s = lax.dot_general(q, kbuf[slot].reshape(T, DH), _NT,
                            preferred_element_type=f32) * scale
        m_old = m_scr[...]
        m_new = jnp.maximum(m_old, jnp.max(s, axis=1, keepdims=True))
        alpha = jnp.exp(m_old - m_new)
        p = jnp.exp(s - m_new)
        l_scr[...] = alpha * l_scr[...] + jnp.sum(p, axis=1, keepdims=True)
        m_scr[...] = m_new
        v_wait(slot)
        pv = jnp.dot(p.astype(bf16), vbuf[slot].reshape(T, DH),
                     preferred_element_type=f32)
        acc_scr[...] = alpha * acc_scr[...] + pv

        @pl.when(c == NCH - 1)
        def _():
            o_h = acc_scr[...] / l_scr[...]
            z = jnp.concatenate(
                [jnp.where(row == 0, o_h, 0.0), jnp.where(row == 1, o_h, 0.0)],
                axis=1).astype(bf16)
            lane = pl.multiple_of(h * (REP * DH), REP * DH)
            attn_scr[...] += lax.dot_general(
                z, wobuf[:, pl.ds(lane, REP * DH)], _NT, preferred_element_type=f32)

        return carry

    lax.fori_loop(0, TOTAL, body, 0)

    attn = jnp.sum(attn_scr[...], axis=0, keepdims=True)
    base = x + attn + (xn + xn * 0.0)
    y = jnp.zeros((ROWS, D), f32)
    for j in range(N_WD):
        wd_wait(j)
        y = y + lax.dot_general(hid_scr[:, j * WD_PIECE:(j + 1) * WD_PIECE], wdbuf[j],
                                _NT, preferred_element_type=f32)
    y = y[0:1] * gate

    out = base + y
    o_ref[0] = out.astype(o_ref.dtype)


@jax.jit
def pallas_parallel_sum__gqa_block_cached__moe_arch_mod__decode_kernel(
    A_x: jax.Array,
    A_k_cache: jax.Array,
    A_v_cache: jax.Array,
    A_wq: jax.Array,
    A_wo: jax.Array,
    B_x: jax.Array,
    B_w_r: jax.Array,
    B_w_gate: jax.Array,
    B_w_up: jax.Array,
    B_w_down: jax.Array,
):
    del B_x
    bf16 = jnp.bfloat16
    f32 = jnp.float32
    any_spec = pl.BlockSpec(memory_space=pl.ANY)
    scratch = [
        pltpu.VMEM((1, 1, D), bf16),
        pltpu.VMEM((D,), bf16),
        pltpu.VMEM((D, HQ * DH), bf16),
        pltpu.VMEM((D, HQ * DH), bf16),
        pltpu.VMEM((D, F), bf16),
        pltpu.VMEM((D, F), bf16),
        pltpu.VMEM((N_WD, D, WD_PIECE), bf16),
        pltpu.VMEM((NBUF, NSEG, PER, DH), bf16),
        pltpu.VMEM((NBUF, NSEG, PER, DH), bf16),
        pltpu.VMEM((HKV, ROWS, DH), bf16),
        pltpu.VMEM((ROWS, F), bf16),
        pltpu.VMEM((ROWS, D), f32),
        pltpu.VMEM((ROWS, 1), f32),
        pltpu.VMEM((ROWS, 1), f32),
        pltpu.VMEM((ROWS, DH), f32),
        pltpu.SemaphoreType.DMA((2, NBUF)),
        pltpu.SemaphoreType.DMA((6,)),
        pltpu.SemaphoreType.DMA((N_WD,)),
    ]
    return pl.pallas_call(
        _kernel,
        out_shape=jax.ShapeDtypeStruct((1, 1, D), bf16),
        in_specs=[any_spec] * 9,
        out_specs=pl.BlockSpec(memory_space=pltpu.VMEM),
        scratch_shapes=scratch,
        compiler_params=pltpu.CompilerParams(vmem_limit_bytes=64 * 1024 * 1024),
    )(A_x, A_k_cache.reshape(HKV, NSEG, SEG, DH), A_v_cache.reshape(HKV, NSEG, SEG, DH),
      A_wq, A_wo.T, B_w_r, B_w_gate, B_w_up, B_w_down.T)
```

```python
import functools

import jax
import jax.numpy as jnp
from jax import lax
import jax.experimental.pallas as pl
import jax.experimental.pallas.tpu as pltpu

D = 448
HQ = 16
HKV = 8
REP = HQ // HKV
SK = 65536
DH = 256
F = 1792
ROWS = 8
EPS = 1e-5

T = 2048
NBUF = 4
NSEG = 8
TP = 8
SEG = SK // NSEG
PER = T // NSEG
NCH = SK // T
TOTAL = HKV * NCH
assert NBUF >= 2
WD_PIECE = 256
N_WD = F // WD_PIECE

_NT = (((1,), (1,)), ((), ()))


def _kernel(x_hbm, k_hbm, v_hbm, wq_hbm, wot_hbm, wr_hbm, wg_hbm, wu_hbm, wdt_hbm,
            o_ref,
            xbuf, wrbuf, wqbuf, wobuf, wgbuf, wubuf, wdbuf, kbuf, vbuf,
            q_scr, hid_scr, attn_scr, m_scr, l_scr, acc_scr,
            kv_sems, w_sems, wd_sems):
    f32 = jnp.float32
    bf16 = jnp.bfloat16

    def kv_start(i, slot):
        h = i // NCH
        base = (i % NCH) * PER

        def piece(j, c2):
            off = pl.multiple_of(j * TP, TP)
            src = pl.multiple_of(base + off, TP)
            pltpu.make_async_copy(v_hbm.at[h, :, pl.ds(src, TP)],
                                  vbuf.at[slot, :, pl.ds(off, TP)],
                                  kv_sems.at[1, slot]).start(priority=1)
            pltpu.make_async_copy(k_hbm.at[h, :, pl.ds(src, TP)],
                                  kbuf.at[slot, :, pl.ds(off, TP)],
                                  kv_sems.at[0, slot]).start(priority=0)
            return c2

        lax.fori_loop(0, PER // TP, piece, 0)

    def k_wait(slot):
        pltpu.make_async_copy(kbuf.at[slot], kbuf.at[slot], kv_sems.at[0, slot]).wait()

    def v_wait(slot):
        pltpu.make_async_copy(vbuf.at[slot], vbuf.at[slot], kv_sems.at[1, slot]).wait()

    x_cp = pltpu.make_async_copy(x_hbm, xbuf, w_sems.at[0])
    wr_cp = pltpu.make_async_copy(wr_hbm, wrbuf, w_sems.at[1])

    def wqo_start():
        def piece(j, c2):
            lane = pl.multiple_of((j % 2) * (HQ * DH // 2), 128)
            for qd in range(4):
                r = pl.multiple_of(qd * (D // 4) + (j // 2) * 8, 8)
                idx = (pl.ds(r, 8), pl.ds(lane, HQ * DH // 2))
                pltpu.make_async_copy(wot_hbm.at[idx], wobuf.at[idx],
                                      w_sems.at[3]).start(priority=1)
                pltpu.make_async_copy(wq_hbm.at[idx], wqbuf.at[idx],
                                      w_sems.at[2]).start(priority=0)
            return c2

        lax.fori_loop(0, 2 * (D // 4 // 8), piece, 0)

    wq_cp = pltpu.make_async_copy(wqbuf, wqbuf, w_sems.at[2])
    wo_cp = pltpu.make_async_copy(wobuf, wobuf, w_sems.at[3])

    def wgu_start():
        def piece(j, c2):
            for qd in range(4):
                r = pl.multiple_of(qd * (D // 4) + j * 8, 8)
                pltpu.make_async_copy(wu_hbm.at[pl.ds(r, 8)], wubuf.at[pl.ds(r, 8)],
                                      w_sems.at[5]).start(priority=1)
                pltpu.make_async_copy(wg_hbm.at[pl.ds(r, 8)], wgbuf.at[pl.ds(r, 8)],
                                      w_sems.at[4]).start(priority=0)
            return c2

        lax.fori_loop(0, D // 4 // 8, piece, 0)

    wg_cp = pltpu.make_async_copy(wgbuf, wgbuf, w_sems.at[4])
    wu_cp = pltpu.make_async_copy(wubuf, wubuf, w_sems.at[5])

    def wd_start():
        def group(g, c2):
            lane = pl.multiple_of(g * WD_PIECE, WD_PIECE)
            pltpu.make_async_copy(wdt_hbm.at[:, pl.ds(lane, WD_PIECE)], wdbuf.at[g],
                                  wd_sems.at[g]).start(priority=1)
            return c2

        lax.fori_loop(0, N_WD, group, 0)

    def wd_wait(g):
        pltpu.make_async_copy(wdbuf.at[g], wdbuf.at[g], wd_sems.at[g]).wait()

    x_cp.start()
    wr_cp.start()
    wqo_start()
    wgu_start()

    x_cp.wait()
    x = xbuf[0].astype(f32)
    mean = jnp.mean(x, axis=-1, keepdims=True)
    xc = x - mean
    var = jnp.mean(xc * xc, axis=-1, keepdims=True)
    xn = xc / jnp.sqrt(var + EPS)
    xn_rows = jnp.broadcast_to(xn, (ROWS, D)).astype(bf16)

    row = lax.broadcasted_iota(jnp.int32, (ROWS, DH), 0)
    wq_cp.wait()
    for h in range(HKV):
        y = jnp.dot(xn_rows, wqbuf[:, h * REP * DH:(h + 1) * REP * DH],
                    preferred_element_type=f32)
        q_h = jnp.where(row == 0, y[:, :DH],
                        jnp.where(row == 1, y[:, DH:], 0.0))
        q_scr[h] = q_h.astype(bf16)

    for i in range(NBUF - 1):
        kv_start(i, i)

    wr_cp.wait()
    wr = wrbuf[...].astype(f32).reshape(1, D)
    r = jnp.sum(xn_rows[0:1].astype(f32) * wr, axis=-1, keepdims=True)
    gate = jax.nn.sigmoid(r)
    wg_cp.wait()
    g = jnp.dot(xn_rows, wgbuf[...], preferred_element_type=f32)
    wu_cp.wait()
    u = jnp.dot(xn_rows, wubuf[...], preferred_element_type=f32)
    hid_scr[...] = (g * jax.nn.sigmoid(g) * u).astype(bf16)
    attn_scr[...] = jnp.zeros(attn_scr.shape, f32)
    wo_cp.wait()

    scale = DH ** -0.5

    def body(i, carry):
        slot = i % NBUF
        h = i // NCH
        c = i % NCH
        nxt = i + NBUF - 1

        @pl.when(nxt < TOTAL)
        def _():
            kv_start(nxt, nxt % NBUF)

        @pl.when(nxt == TOTAL)
        def _():
            wd_start()

        @pl.when(c == 0)
        def _():
            m_scr[...] = jnp.full(m_scr.shape, -jnp.inf, f32)
            l_scr[...] = jnp.zeros(l_scr.shape, f32)
            acc_scr[...] = jnp.zeros(acc_scr.shape, f32)

        q = q_scr[h]
        k_wait(slot)
        s = lax.dot_general(q, kbuf[slot].reshape(T, DH), _NT,
                            preferred_element_type=f32) * scale
        m_old = m_scr[...]
        m_new = jnp.maximum(m_old, jnp.max(s, axis=1, keepdims=True))
        alpha = jnp.exp(m_old - m_new)
        p = jnp.exp(s - m_new)
        l_scr[...] = alpha * l_scr[...] + jnp.sum(p, axis=1, keepdims=True)
        m_scr[...] = m_new
        v_wait(slot)
        pv = jnp.dot(p.astype(bf16), vbuf[slot].reshape(T, DH),
                     preferred_element_type=f32)
        acc_scr[...] = alpha * acc_scr[...] + pv

        @pl.when(c == NCH - 1)
        def _():
            o_h = acc_scr[...] / l_scr[...]
            z = jnp.concatenate(
                [jnp.where(row == 0, o_h, 0.0), jnp.where(row == 1, o_h, 0.0)],
                axis=1).astype(bf16)
            lane = pl.multiple_of(h * (REP * DH), REP * DH)
            attn_scr[...] += lax.dot_general(
                z, wobuf[:, pl.ds(lane, REP * DH)], _NT, preferred_element_type=f32)

        return carry

    lax.fori_loop(0, TOTAL, body, 0)

    attn = jnp.sum(attn_scr[...], axis=0, keepdims=True)
    base = x + attn + (xn + xn * 0.0)
    y = jnp.zeros((ROWS, D), f32)
    for j in range(N_WD):
        wd_wait(j)
        y = y + lax.dot_general(hid_scr[:, j * WD_PIECE:(j + 1) * WD_PIECE], wdbuf[j],
                                _NT, preferred_element_type=f32)
    y = y[0:1] * gate

    out = base + y
    o_ref[0] = out.astype(o_ref.dtype)


@jax.jit
def pallas_parallel_sum__gqa_block_cached__moe_arch_mod__decode_kernel(
    A_x: jax.Array,
    A_k_cache: jax.Array,
    A_v_cache: jax.Array,
    A_wq: jax.Array,
    A_wo: jax.Array,
    B_x: jax.Array,
    B_w_r: jax.Array,
    B_w_gate: jax.Array,
    B_w_up: jax.Array,
    B_w_down: jax.Array,
):
    del B_x
    bf16 = jnp.bfloat16
    f32 = jnp.float32
    any_spec = pl.BlockSpec(memory_space=pl.ANY)
    scratch = [
        pltpu.VMEM((1, 1, D), bf16),
        pltpu.VMEM((D,), bf16),
        pltpu.VMEM((D, HQ * DH), bf16),
        pltpu.VMEM((D, HQ * DH), bf16),
        pltpu.VMEM((D, F), bf16),
        pltpu.VMEM((D, F), bf16),
        pltpu.VMEM((N_WD, D, WD_PIECE), bf16),
        pltpu.VMEM((NBUF, NSEG, PER, DH), bf16),
        pltpu.VMEM((NBUF, NSEG, PER, DH), bf16),
        pltpu.VMEM((HKV, ROWS, DH), bf16),
        pltpu.VMEM((ROWS, F), bf16),
        pltpu.VMEM((ROWS, D), f32),
        pltpu.VMEM((ROWS, 1), f32),
        pltpu.VMEM((ROWS, 1), f32),
        pltpu.VMEM((ROWS, DH), f32),
        pltpu.SemaphoreType.DMA((2, NBUF)),
        pltpu.SemaphoreType.DMA((6,)),
        pltpu.SemaphoreType.DMA((N_WD,)),
    ]
    return pl.pallas_call(
        _kernel,
        out_shape=jax.ShapeDtypeStruct((1, 1, D), bf16),
        in_specs=[any_spec] * 9,
        out_specs=pl.BlockSpec(memory_space=pltpu.VMEM),
        scratch_shapes=scratch,
        compiler_params=pltpu.CompilerParams(vmem_limit_bytes=64 * 1024 * 1024),
    )(A_x, A_k_cache.reshape(HKV, NSEG, SEG, DH), A_v_cache.reshape(HKV, NSEG, SEG, DH),
      A_wq, A_wo.T, B_w_r, B_w_gate, B_w_up, B_w_down.T)
```

```python
import jax
import jax.numpy as jnp
from jax import lax
import jax.experimental.pallas as pl
import jax.experimental.pallas.tpu as pltpu

D = 448
HQ = 16
HKV = 8
REP = HQ // HKV
SK = 65536
DH = 256
F = 1792
ROWS = 8
EPS = 1e-5

T = 2048
NBUF = 4
NSEG = 8
TP = 8
SEG = SK // NSEG
PER = T // NSEG
NCH = SK // T
TOTAL = HKV * NCH
assert NBUF >= 2
WD_PIECE = 256
N_WD = F // WD_PIECE

_NT = (((1,), (1,)), ((), ()))


def _kernel_body(x_hbm, k_hbm, v_hbm, wq_hbm, wot_hbm, wr_hbm, wg_hbm, wu_hbm, wdt_hbm,
                 o_ref,
                 xbuf, wrbuf, wqbuf, wobuf, wgbuf, wubuf, wdbuf, kbuf, vbuf,
                 q_scr, hid_scr, attn_scr, m_scr, l_scr, acc_scr,
                 kv_sems, w_sems, wd_sems):
    f32 = jnp.float32
    bf16 = jnp.bfloat16

    def kv_start(i, slot):
        h = i // NCH
        base = (i % NCH) * PER

        def piece(j, c2):
            off = pl.multiple_of(j * TP, TP)
            src = pl.multiple_of(base + off, TP)
            pltpu.make_async_copy(v_hbm.at[h, :, pl.ds(src, TP)],
                                  vbuf.at[slot, :, pl.ds(off, TP)],
                                  kv_sems.at[1, slot]).start(priority=1)
            pltpu.make_async_copy(k_hbm.at[h, :, pl.ds(src, TP)],
                                  kbuf.at[slot, :, pl.ds(off, TP)],
                                  kv_sems.at[0, slot]).start(priority=0)
            return c2

        lax.fori_loop(0, PER // TP, piece, 0)

    def k_wait(slot):
        pltpu.make_async_copy(kbuf.at[slot], kbuf.at[slot], kv_sems.at[0, slot]).wait()

    def v_wait(slot):
        pltpu.make_async_copy(vbuf.at[slot], vbuf.at[slot], kv_sems.at[1, slot]).wait()

    x_cp = pltpu.make_async_copy(x_hbm, xbuf, w_sems.at[0])
    wr_cp = pltpu.make_async_copy(wr_hbm, wrbuf, w_sems.at[1])

    def wqo_start():
        def piece(j, c2):
            lane = pl.multiple_of((j % 2) * (HQ * DH // 2), 128)
            for qd in range(4):
                r = pl.multiple_of(qd * (D // 4) + (j // 2) * 8, 8)
                idx = (pl.ds(r, 8), pl.ds(lane, HQ * DH // 2))
                pltpu.make_async_copy(wot_hbm.at[idx], wobuf.at[idx],
                                      w_sems.at[3]).start(priority=1)
                pltpu.make_async_copy(wq_hbm.at[idx], wqbuf.at[idx],
                                      w_sems.at[2]).start(priority=0)
            return c2

        lax.fori_loop(0, 2 * (D // 4 // 8), piece, 0)

    wq_cp = pltpu.make_async_copy(wqbuf, wqbuf, w_sems.at[2])
    wo_cp = pltpu.make_async_copy(wobuf, wobuf, w_sems.at[3])

    def wgu_start():
        def piece(j, c2):
            for qd in range(4):
                r = pl.multiple_of(qd * (D // 4) + j * 8, 8)
                pltpu.make_async_copy(wu_hbm.at[pl.ds(r, 8)], wubuf.at[pl.ds(r, 8)],
                                      w_sems.at[5]).start(priority=1)
                pltpu.make_async_copy(wg_hbm.at[pl.ds(r, 8)], wgbuf.at[pl.ds(r, 8)],
                                      w_sems.at[4]).start(priority=0)
            return c2

        lax.fori_loop(0, D // 4 // 8, piece, 0)

    wg_cp = pltpu.make_async_copy(wgbuf, wgbuf, w_sems.at[4])
    wu_cp = pltpu.make_async_copy(wubuf, wubuf, w_sems.at[5])

    def wd_start():
        def group(g, c2):
            lane = pl.multiple_of(g * WD_PIECE, WD_PIECE)
            pltpu.make_async_copy(wdt_hbm.at[:, pl.ds(lane, WD_PIECE)], wdbuf.at[g],
                                  wd_sems.at[g]).start(priority=1)
            return c2

        lax.fori_loop(0, N_WD, group, 0)

    def wd_wait(g):
        pltpu.make_async_copy(wdbuf.at[g], wdbuf.at[g], wd_sems.at[g]).wait()

    x_cp.start()
    wr_cp.start()
    wqo_start()
    wgu_start()

    x_cp.wait()
    x = xbuf[0].astype(f32)
    mean = jnp.mean(x, axis=-1, keepdims=True)
    xc = x - mean
    var = jnp.mean(xc * xc, axis=-1, keepdims=True)
    xn = xc / jnp.sqrt(var + EPS)
    xn_rows = jnp.broadcast_to(xn, (ROWS, D)).astype(bf16)

    row = lax.broadcasted_iota(jnp.int32, (ROWS, DH), 0)
    wq_cp.wait()
    for h in range(HKV):
        y = jnp.dot(xn_rows, wqbuf[:, h * REP * DH:(h + 1) * REP * DH],
                    preferred_element_type=f32)
        q_h = jnp.where(row == 0, y[:, :DH],
                        jnp.where(row == 1, y[:, DH:], 0.0))
        q_scr[h] = q_h.astype(bf16)

    for i in range(NBUF - 1):
        kv_start(i, i)

    wr_cp.wait()
    wr = wrbuf[...].astype(f32).reshape(1, D)
    r = jnp.sum(xn_rows[0:1].astype(f32) * wr, axis=-1, keepdims=True)
    gate = jax.nn.sigmoid(r)
    wg_cp.wait()
    g = jnp.dot(xn_rows, wgbuf[...], preferred_element_type=f32)
    wu_cp.wait()
    u = jnp.dot(xn_rows, wubuf[...], preferred_element_type=f32)
    hid_scr[...] = (g * jax.nn.sigmoid(g) * u).astype(bf16)
    attn_scr[...] = jnp.zeros(attn_scr.shape, f32)
    wo_cp.wait()

    scale = DH ** -0.5

    def body(i, carry):
        slot = i % NBUF
        h = i // NCH
        c = i % NCH
        nxt = i + NBUF - 1

        @pl.when(nxt < TOTAL)
        def _():
            kv_start(nxt, nxt % NBUF)

        @pl.when(nxt == TOTAL)
        def _():
            wd_start()

        @pl.when(c == 0)
        def _():
            m_scr[...] = jnp.full(m_scr.shape, -jnp.inf, f32)
            l_scr[...] = jnp.zeros(l_scr.shape, f32)
            acc_scr[...] = jnp.zeros(acc_scr.shape, f32)

        q = q_scr[h]
        k_wait(slot)
        s = lax.dot_general(q, kbuf[slot].reshape(T, DH), _NT,
                            preferred_element_type=f32) * scale
        m_old = m_scr[...]
        m_new = jnp.maximum(m_old, jnp.max(s, axis=1, keepdims=True))
        alpha = jnp.exp(m_old - m_new)
        p = jnp.exp(s - m_new)
        l_scr[...] = alpha * l_scr[...] + jnp.sum(p, axis=1, keepdims=True)
        m_scr[...] = m_new
        v_wait(slot)
        pv = jnp.dot(p.astype(bf16), vbuf[slot].reshape(T, DH),
                     preferred_element_type=f32)
        acc_scr[...] = alpha * acc_scr[...] + pv

        @pl.when(c == NCH - 1)
        def _():
            o_h = acc_scr[...] / l_scr[...]
            z = jnp.concatenate(
                [jnp.where(row == 0, o_h, 0.0), jnp.where(row == 1, o_h, 0.0)],
                axis=1).astype(bf16)
            lane = pl.multiple_of(h * (REP * DH), REP * DH)
            attn_scr[...] += lax.dot_general(
                z, wobuf[:, pl.ds(lane, REP * DH)], _NT, preferred_element_type=f32)

        return carry

    lax.fori_loop(0, TOTAL, body, 0)

    attn = jnp.sum(attn_scr[...], axis=0, keepdims=True)
    base = x + attn + (xn + xn * 0.0)
    y = jnp.zeros((ROWS, D), f32)
    for j in range(N_WD):
        wd_wait(j)
        y = y + lax.dot_general(hid_scr[:, j * WD_PIECE:(j + 1) * WD_PIECE], wdbuf[j],
                                _NT, preferred_element_type=f32)
    y = y[0:1] * gate

    out = base + y
    o_ref[0] = out.astype(o_ref.dtype)


def _kernel(*refs):
    pl.run_scoped(
        lambda *sems: _kernel_body(*refs, *sems),
        pltpu.SemaphoreType.DMA((2, NBUF)),
        pltpu.SemaphoreType.DMA((6,)),
        pltpu.SemaphoreType.DMA((N_WD,)),
    )


@jax.jit
def pallas_parallel_sum__gqa_block_cached__moe_arch_mod__decode_kernel(
    A_x: jax.Array,
    A_k_cache: jax.Array,
    A_v_cache: jax.Array,
    A_wq: jax.Array,
    A_wo: jax.Array,
    B_x: jax.Array,
    B_w_r: jax.Array,
    B_w_gate: jax.Array,
    B_w_up: jax.Array,
    B_w_down: jax.Array,
):
    del B_x
    bf16 = jnp.bfloat16
    f32 = jnp.float32
    any_spec = pl.BlockSpec(memory_space=pl.ANY)
    scratch = [
        pltpu.VMEM((1, 1, D), bf16),
        pltpu.VMEM((D,), bf16),
        pltpu.VMEM((D, HQ * DH), bf16),
        pltpu.VMEM((D, HQ * DH), bf16),
        pltpu.VMEM((D, F), bf16),
        pltpu.VMEM((D, F), bf16),
        pltpu.VMEM((N_WD, D, WD_PIECE), bf16),
        pltpu.VMEM((NBUF, NSEG, PER, DH), bf16),
        pltpu.VMEM((NBUF, NSEG, PER, DH), bf16),
        pltpu.VMEM((HKV, ROWS, DH), bf16),
        pltpu.VMEM((ROWS, F), bf16),
        pltpu.VMEM((ROWS, D), f32),
        pltpu.VMEM((ROWS, 1), f32),
        pltpu.VMEM((ROWS, 1), f32),
        pltpu.VMEM((ROWS, DH), f32),
    ]
    return pl.pallas_call(
        _kernel,
        out_shape=jax.ShapeDtypeStruct((1, 1, D), bf16),
        in_specs=[any_spec] * 9,
        out_specs=pl.BlockSpec(memory_space=pltpu.VMEM),
        scratch_shapes=scratch,
        compiler_params=pltpu.CompilerParams(vmem_limit_bytes=64 * 1024 * 1024),
    )(A_x, A_k_cache.reshape(HKV, NSEG, SEG, DH), A_v_cache.reshape(HKV, NSEG, SEG, DH),
      A_wq, A_wo.T, B_w_r, B_w_gate, B_w_up, B_w_down.T)
```
